```python
import os as _os
_os.environ.setdefault("JAX_PLATFORMS", "cpu")
import jax
import jax.numpy as jnp

def _softmax(x, axis=-1):
    return jax.nn.softmax(x, axis=axis)
def _gelu(x):
    return jax.nn.gelu(x, approximate=True)
def _silu(x):
    return jax.nn.silu(x)
def _sigmoid(x):
    return jax.nn.sigmoid(x)
def _layernorm(x, axis=-1, eps=1e-5):
    m = jnp.mean(x, axis=axis, keepdims=True)
    v = jnp.var(x, axis=axis, keepdims=True)
    return (x - m) / jnp.sqrt(v + eps)
def _scatter_add(tgt, idx, src, axis=0):
    return tgt.at[idx].add(src)
def _segment_sum(src, seg, n):
    return jax.ops.segment_sum(src, seg, n)
class _Rng:
    def __init__(self, key):
        self._k = key
    def _next(self):
        self._k, sub = jax.random.split(self._k)
        return sub
    def normal(self, shape):
        return jax.random.normal(self._next(), shape, dtype=jnp.bfloat16)
    def randint(self, lo, hi, shape):
        return jax.random.randint(self._next(), shape, lo, hi, dtype=jnp.int32)
    def uniform(self, shape, lo=0.0, hi=1.0):
        return jax.random.uniform(self._next(), shape, jnp.bfloat16, lo, hi)
    def permutation(self, n):
        return jax.random.permutation(self._next(), n)


kernel_name = 'standalone__sliding_local_fixed_window__prompt'

def setup_inputs():
    _rng = _Rng(jax.random.key(int.from_bytes(__import__("os").urandom(4), "little")))
    _w = (lambda a: (lambda t: t.astype(jnp.bfloat16) if jnp.issubdtype(t.dtype, jnp.floating) else t)(jnp.asarray(a)))
    B, H, S, D = 1, 32, 2048, 128
    return {
        "q": _w((lambda *s: _rng.normal(s) * 0.4)(B, H, S, D)),
        "k": _w((lambda *s: _rng.normal(s) * 0.4)(B, H, S, D)),
        "v": _w((lambda *s: _rng.normal(s) * 0.05)(B, H, S, D)),
    }

def reference(q, k, v):
    B, H, S, D = q.shape
    w = 32
    pos = jnp.arange(S)
    rel = pos[:, None] - pos[None, :]
    mask = (rel >= 0) & (rel < w)
    scores = jnp.einsum("bhqd,bhkd->bhqk", q, k) * (D ** -0.5)
    scores = jnp.where(mask[None, None], scores, (lambda x, dt: x.astype(dt))(jnp.array(-1e9), q.dtype))
    p = _softmax(scores, axis=-1)
    return jnp.einsum("bhqk,bhkd->bhqd", p, v)
```

```python
import math

import jax
from jax import lax
import jax.experimental.pallas as pl
import jax.experimental.pallas.tpu as pltpu
import jax.numpy as jnp

_WINDOW = 32
_TILE = 128
_STEP = _TILE - _WINDOW
_NEG = -1e30


def _attend(q, k, v, offset, scale_log2):
    s = lax.dot_general(
        q, k, (((1,), (1,)), ((), ())), preferred_element_type=jnp.float32
    )
    rel = (
        lax.broadcasted_iota(jnp.int32, s.shape, 0)
        - lax.broadcasted_iota(jnp.int32, s.shape, 1)
        + offset
    )
    s = jnp.where((rel >= 0) & (rel < _WINDOW), s, _NEG)
    m = jnp.max(s, axis=1, keepdims=True)
    p = jnp.exp2((s - m) * scale_log2)
    l = jnp.sum(p, axis=1, keepdims=True)
    o = jnp.dot(p.astype(v.dtype), v, preferred_element_type=jnp.float32)
    return o * (1.0 / l)


@jax.jit
def pallas_standalone__sliding_local_fixed_window__prompt_kernel(
    q: jax.Array,
    k: jax.Array,
    v: jax.Array,
):
    B, H, S, D = q.shape
    heads = B * H
    rows = heads * S
    assert S >= _TILE and (S - _TILE) % _STEP == 0
    scale_log2 = D**-0.5 * math.log2(math.e)

    n_chunks = 4
    n_early = 4
    tail = 1024
    assert heads % n_chunks == 0
    hpc = heads // n_chunks
    early_heads = heads - hpc
    wb = [early_heads * i // n_early * S for i in range(n_early + 1)] + [rows]

    def kernel(q_hbm, k_hbm, v_hbm, o_hbm, qb, kb, vb, ob, rsem, wsem):
        def reads(slot, start, size):
            sl = pl.ds(start, size)
            return [
                pltpu.make_async_copy(src.at[sl], dst.at[sl], rsem.at[slot, j])
                for j, (src, dst) in enumerate(((q_hbm, qb), (k_hbm, kb), (v_hbm, vb)))
            ]

        chunks = [
            reads(c, c * hpc * S, hpc * S - (tail if c == n_chunks - 1 else 0))
            for c in range(n_chunks)
        ]
        tails = reads(n_chunks, rows - tail, tail)
        writes = [
            pltpu.make_async_copy(
                ob.at[pl.ds(a, b - a)], o_hbm.at[pl.ds(a, b - a)], wsem.at[i]
            )
            for i, (a, b) in enumerate(zip(wb[:-1], wb[1:]))
        ]

        for group in chunks + [tails]:
            for cp in group:
                cp.start()

        def head(h, carry):
            for c in range(n_chunks):

                @pl.when(h == c * hpc)
                def _():
                    for cp in chunks[c]:
                        cp.wait()
                    if c == n_chunks - 1:
                        for i in range(n_early):
                            writes[i].start(priority=i % 2)
                        for cp in tails:
                            cp.wait()

            sl = pl.ds(pl.multiple_of(h * S, S), S)
            qh, kh, vh, oh = qb.at[sl], kb.at[sl], vb.at[sl], ob.at[sl]
            for k0 in range(0, S - _TILE + 1, _STEP):
                offset = _WINDOW if k0 else 0
                qs, ks = slice(k0 + offset, k0 + _TILE), slice(k0, k0 + _TILE)
                o = _attend(qh[qs, :], kh[ks, :], vh[ks, :], offset, scale_log2)
                oh[qs, :] = o.astype(oh.dtype)
            return carry

        lax.fori_loop(0, heads, head, None)
        writes[-1].start()
        for cp in writes:
            cp.wait()

    hbm = pl.BlockSpec(memory_space=pl.ANY)
    out = pl.pallas_call(
        kernel,
        in_specs=[hbm] * 3,
        out_specs=hbm,
        out_shape=jax.ShapeDtypeStruct((rows, D), q.dtype),
        scratch_shapes=[pltpu.VMEM((rows, D), q.dtype)] * 4
        + [
            pltpu.SemaphoreType.DMA((n_chunks + 1, 3)),
            pltpu.SemaphoreType.DMA((n_early + 1,)),
        ],
        compiler_params=pltpu.CompilerParams(vmem_limit_bytes=100 * 2**20),
    )(q.reshape(rows, D), k.reshape(rows, D), v.reshape(rows, D))
    return out.reshape(q.shape)
```

```python
import math

import jax
from jax import lax
import jax.experimental.pallas as pl
import jax.experimental.pallas.tpu as pltpu
import jax.numpy as jnp

_WINDOW = 32
_TILE = 128
_STEP = _TILE - _WINDOW
_MASKED = -1e30
_WRITE_ROWS = 256
_TAIL_ROWS = 512


def _attend(q, k, v, offset, scale_log2):
    s = lax.dot_general(
        q, k, (((1,), (1,)), ((), ())), preferred_element_type=jnp.float32
    )
    rel = (
        lax.broadcasted_iota(jnp.int32, s.shape, 0)
        - lax.broadcasted_iota(jnp.int32, s.shape, 1)
        + offset
    )
    s = jnp.where((rel >= 0) & (rel < _WINDOW), s, _MASKED)
    m = jnp.max(s, axis=1, keepdims=True)
    p = jnp.exp2((s - m) * scale_log2)
    l = jnp.sum(p, axis=1, keepdims=True)
    o = jnp.dot(p.astype(v.dtype), v, preferred_element_type=jnp.float32)
    return o * (1.0 / l)


@jax.jit
def pallas_standalone__sliding_local_fixed_window__prompt_kernel(
    q: jax.Array,
    k: jax.Array,
    v: jax.Array,
):
    B, H, S, D = q.shape
    heads = B * H
    rows = heads * S
    assert S >= _TILE and (S - _TILE) % _STEP == 0 and S % _WRITE_ROWS == 0
    scale_log2 = D**-0.5 * math.log2(math.e)

    bounds = [0, heads * 13 // 32, heads * 22 // 32, heads]
    last = len(bounds) - 2
    pieces = S // _WRITE_ROWS

    def kernel(q_hbm, k_hbm, v_hbm, o_hbm, qb, kb, vb, ob, rsem, wsem):
        def reads(slot, start, stop):
            sl = pl.ds(start, stop - start)
            return [
                pltpu.make_async_copy(src.at[sl], dst.at[sl], rsem.at[slot, j])
                for j, (src, dst) in enumerate(((q_hbm, qb), (k_hbm, kb), (v_hbm, vb)))
            ]

        def writes(slot, start, stop):
            copies = []
            for g in range(pieces):
                sl = (pl.ds(start, stop - start), pl.ds(g * _WRITE_ROWS, _WRITE_ROWS))
                copies.append(
                    pltpu.make_async_copy(ob.at[sl], o_hbm.at[sl], wsem.at[slot, g])
                )
            return copies

        chunks = [
            reads(c, bounds[c] * S, min(bounds[c + 1] * S, rows - _TAIL_ROWS))
            for c in range(last + 1)
        ]
        tail = reads(last + 1, rows - _TAIL_ROWS, rows)
        early_writes = writes(0, 0, bounds[last])
        late_writes = writes(1, bounds[last], heads)

        for group in chunks + [tail]:
            for cp in group:
                cp.start()

        def head(h, carry):
            for c, chunk in enumerate(chunks):

                @pl.when(h == bounds[c])
                def _():
                    for cp in chunk:
                        cp.wait()
                    if c == last:
                        for cp in early_writes:
                            cp.start()
                        for cp in tail:
                            cp.wait()

            sl = pl.ds(pl.multiple_of(h * S, S), S)
            qh, kh, vh, oh = qb.at[sl], kb.at[sl], vb.at[sl], ob.at[h]
            for k0 in range(0, S - _TILE + 1, _STEP):
                offset = _WINDOW if k0 else 0
                qs, ks = slice(k0 + offset, k0 + _TILE), slice(k0, k0 + _TILE)
                o = _attend(qh[qs, :], kh[ks, :], vh[ks, :], offset, scale_log2)
                oh[qs, :] = o.astype(oh.dtype)
            return carry

        lax.fori_loop(0, heads, head, None)
        for cp in late_writes:
            cp.start()
        for cp in early_writes + late_writes:
            cp.wait()

    hbm = pl.BlockSpec(memory_space=pl.ANY)
    out = pl.pallas_call(
        kernel,
        in_specs=[hbm] * 3,
        out_specs=hbm,
        out_shape=jax.ShapeDtypeStruct((heads, S, D), q.dtype),
        scratch_shapes=[
            pltpu.VMEM((rows, D), q.dtype),
            pltpu.VMEM((rows, D), k.dtype),
            pltpu.VMEM((rows, D), v.dtype),
            pltpu.VMEM((heads, S, D), q.dtype),
            pltpu.SemaphoreType.DMA((last + 2, 3)),
            pltpu.SemaphoreType.DMA((2, pieces)),
        ],
        compiler_params=pltpu.CompilerParams(vmem_limit_bytes=100 * 2**20),
    )(q.reshape(rows, D), k.reshape(rows, D), v.reshape(rows, D))
    return out.reshape(q.shape)
```

```python
import math

import jax
from jax import lax
import jax.experimental.pallas as pl
import jax.experimental.pallas.tpu as pltpu
import jax.numpy as jnp

_WINDOW = 32
_TILE = 128
_STEP = _TILE - _WINDOW
_MASKED = -1e30
_WRITE_PIECES = 14
_SUBLANES = 16
_TAIL_ROWS = 512


def _attend(q, k, v, offset, scale_log2):
    s = lax.dot_general(
        q, k, (((1,), (1,)), ((), ())), preferred_element_type=jnp.float32
    )
    rel = (
        lax.broadcasted_iota(jnp.int32, s.shape, 0)
        - lax.broadcasted_iota(jnp.int32, s.shape, 1)
        + offset
    )
    s = jnp.where((rel >= 0) & (rel < _WINDOW), s, _MASKED)
    m = jnp.max(s, axis=1, keepdims=True)
    p = jnp.exp2((s - m) * scale_log2)
    l = jnp.sum(p, axis=1, keepdims=True)
    o = jnp.dot(p.astype(v.dtype), v, preferred_element_type=jnp.float32)
    return o * (1.0 / l)


@jax.jit
def pallas_standalone__sliding_local_fixed_window__prompt_kernel(
    q: jax.Array,
    k: jax.Array,
    v: jax.Array,
):
    B, H, S, D = q.shape
    heads = B * H
    rows = heads * S
    assert S >= _TILE and (S - _TILE) % _STEP == 0
    scale_log2 = D**-0.5 * math.log2(math.e)

    bounds = [0, heads * 14 // 32, heads * 23 // 32, heads]
    last = len(bounds) - 2
    cuts = [
        S // _SUBLANES * g // _WRITE_PIECES * _SUBLANES
        for g in range(_WRITE_PIECES + 1)
    ]

    def kernel(q_hbm, k_hbm, v_hbm, o_hbm, qb, kb, vb, ob, rsem, wsem):
        def reads(slot, start, stop):
            sl = pl.ds(start, stop - start)
            return [
                pltpu.make_async_copy(src.at[sl], dst.at[sl], rsem.at[slot, j])
                for j, (src, dst) in enumerate(((q_hbm, qb), (k_hbm, kb), (v_hbm, vb)))
            ]

        def writes(slot, start, stop):
            copies = []
            for g in range(_WRITE_PIECES):
                sl = (pl.ds(start, stop - start), pl.ds(cuts[g], cuts[g + 1] - cuts[g]))
                copies.append(
                    pltpu.make_async_copy(ob.at[sl], o_hbm.at[sl], wsem.at[slot, g])
                )
            return copies

        chunks = [
            reads(c, bounds[c] * S, min(bounds[c + 1] * S, rows - _TAIL_ROWS))
            for c in range(last + 1)
        ]
        tail = reads(last + 1, rows - _TAIL_ROWS, rows)
        early_writes = writes(0, 0, bounds[last])
        late_writes = writes(1, bounds[last], heads)

        for group in chunks + [tail]:
            for cp in group:
                cp.start()

        def head(h, carry):
            for c, chunk in enumerate(chunks):

                @pl.when(h == bounds[c])
                def _():
                    for cp in chunk:
                        cp.wait()
                    if c == last:
                        for cp in early_writes:
                            cp.start()
                        for cp in tail:
                            cp.wait()

            sl = pl.ds(pl.multiple_of(h * S, S), S)
            qh, kh, vh, oh = qb.at[sl], kb.at[sl], vb.at[sl], ob.at[h]
            for k0 in range(0, S - _TILE + 1, _STEP):
                offset = _WINDOW if k0 else 0
                qs, ks = slice(k0 + offset, k0 + _TILE), slice(k0, k0 + _TILE)
                o = _attend(qh[qs, :], kh[ks, :], vh[ks, :], offset, scale_log2)
                oh[qs, :] = o.astype(oh.dtype)
            return carry

        lax.fori_loop(0, heads, head, None)
        for cp in late_writes:
            cp.start()
        for cp in early_writes + late_writes:
            cp.wait()

    hbm = pl.BlockSpec(memory_space=pl.ANY)
    out = pl.pallas_call(
        kernel,
        in_specs=[hbm] * 3,
        out_specs=hbm,
        out_shape=jax.ShapeDtypeStruct((heads, S, D), q.dtype),
        scratch_shapes=[
            pltpu.VMEM((rows, D), q.dtype),
            pltpu.VMEM((rows, D), k.dtype),
            pltpu.VMEM((rows, D), v.dtype),
            pltpu.VMEM((heads, S, D), q.dtype),
            pltpu.SemaphoreType.DMA((last + 2, 3)),
            pltpu.SemaphoreType.DMA((2, _WRITE_PIECES)),
        ],
        compiler_params=pltpu.CompilerParams(vmem_limit_bytes=100 * 2**20),
    )(q.reshape(rows, D), k.reshape(rows, D), v.reshape(rows, D))
    return out.reshape(q.shape)
```
